```python
import jax
import jax.numpy as jnp

def _softmax(x, axis=-1):
    return jax.nn.softmax(x, axis=axis)
def _gelu(x):
    return jax.nn.gelu(x, approximate=True)
def _silu(x):
    return jax.nn.silu(x)
def _sigmoid(x):
    return jax.nn.sigmoid(x)
def _layernorm(x, axis=-1, eps=1e-5):
    m = jnp.mean(x, axis=axis, keepdims=True)
    v = jnp.var(x, axis=axis, keepdims=True)
    return (x - m) / jnp.sqrt(v + eps)
def _scatter_add(tgt, idx, src, axis=0):
    return tgt.at[idx].add(src)
def _segment_sum(src, seg, n):
    return jax.ops.segment_sum(src, seg, n)
class _Rng:
    def __init__(self, key):
        self._k = key
    def _next(self):
        self._k, sub = jax.random.split(self._k)
        return sub
    def normal(self, shape):
        return jax.random.normal(self._next(), shape, dtype=jnp.bfloat16)
    def randint(self, lo, hi, shape):
        return jax.random.randint(self._next(), shape, lo, hi, dtype=jnp.int32)
    def uniform(self, shape, lo=0.0, hi=1.0):
        return jax.random.uniform(self._next(), shape, jnp.bfloat16, lo, hi)
    def permutation(self, n):
        return jax.random.permutation(self._next(), n)


kernel_name = 'sequential_preLN__sliding_block_cached__moe_arch_mod__decode'

def setup_inputs():
    _rng = _Rng(jax.random.key(int.from_bytes(__import__("os").urandom(4), "little")))
    _w = (lambda a: (lambda t: t.astype(jnp.bfloat16) if jnp.issubdtype(t.dtype, jnp.floating) else t)(jnp.asarray(a)))
    def _A_setup():
        B, Sq, D = 1, 1, 640
        Hq, Hkv, Sk, Dh = 32, 32, 32768, 192
        assert Hq % Hkv == 0, (Hq, Hkv)
        return {
            "x": _w((lambda *s: _rng.normal(s) * 0.05)(B, Sq, D)),
            "k_cache": _w((lambda *s: _rng.normal(s) * 0.05)(B, Hkv, Sk, Dh)),
            "v_cache": _w((lambda *s: _rng.normal(s) * 0.05)(B, Hkv, Sk, Dh)),
            "wq": _w((lambda *s: _rng.normal(s) * 0.05)(D, Hq * Dh) * (D ** -0.5)),
            "wo": _w((lambda *s: _rng.normal(s) * 0.05)(Hq * Dh, D) * ((Hq * Dh) ** -0.5)),
        }
    _A_in = _A_setup()

    def _B_setup():
        B, S, D, F, C = 1, 1, 640, 1536, 1
        return {
            "x": _w((lambda *s: _rng.normal(s) * 0.05)(B, S, D)),
            "w_r": _w((lambda *s: _rng.normal(s) * 0.05)(D)),
            "w_gate": _w((lambda *s: _rng.normal(s) * 0.05)(D, F)),
            "w_up": _w((lambda *s: _rng.normal(s) * 0.05)(D, F)),
            "w_down": _w((lambda *s: _rng.normal(s) * 0.05)(F, D)),
        }
    _B_in = _B_setup()

    return {
        "A_x": _A_in["x"],
        "A_k_cache": _A_in["k_cache"],
        "A_v_cache": _A_in["v_cache"],
        "A_wq": _A_in["wq"],
        "A_wo": _A_in["wo"],
        "B_x": _B_in["x"],
        "B_w_r": _B_in["w_r"],
        "B_w_gate": _B_in["w_gate"],
        "B_w_up": _B_in["w_up"],
        "B_w_down": _B_in["w_down"],
    }

def reference(A_x, A_k_cache, A_v_cache, A_wq, A_wo, B_x, B_w_r, B_w_gate, B_w_up, B_w_down):
    def _A_ref(x, k_cache, v_cache, wq, wo):
        B, Sq, D = x.shape
        Hq, Dh = 32, 192
        Hkv, Sk = k_cache.shape[1], k_cache.shape[2]
        W = min(4096, max(256, Sk // 4))
        rep = Hq // Hkv
        q = (lambda x, *d: x.transpose(*d))((x @ wq).reshape(B, Sq, Hq, Dh), 0, 2, 1, 3)
        k = jnp.repeat(k_cache[:, :, Sk - W:, :], rep, axis=1)
        v = jnp.repeat(v_cache[:, :, Sk - W:, :], rep, axis=1)
        scores = jnp.einsum("bhqd,bhkd->bhqk", q, k) * (Dh ** -0.5)
        p = _softmax(scores, axis=-1)
        o = jnp.einsum("bhqk,bhkd->bhqd", p, v)
        return (lambda x, *d: x.transpose(*d))(o, 0, 2, 1, 3).reshape(B, Sq, Hq * Dh) @ wo

    def _B_ref(x, w_r, w_gate, w_up, w_down):
        B, S, D = x.shape
        C = 1
        r = x @ w_r
        idx = jnp.argsort(-r, axis=-1)[:, :C]
        idx_e = jnp.repeat(idx.reshape(B, C, 1), D, axis=2)
        x_sel = jnp.take_along_axis(x, idx_e, axis=1)
        g = _silu(x_sel @ w_gate)
        u = x_sel @ w_up
        y = (g * u) @ w_down
        r_sel = _sigmoid(jnp.take_along_axis(r, idx, axis=1))
        y = y * r_sel.reshape(B, C, 1)
        b_off = (jnp.arange(B) * S).reshape(B, 1)
        flat_idx = (idx + b_off).reshape(B * C)
        zero = (x * 0.0).reshape(B * S, D)
        upd = _scatter_add(zero, flat_idx, y.reshape(B * C, D), axis=0)
        return x + upd.reshape(B, S, D)

    x = A_x
    h = x + _A_ref(_layernorm(x, axis=-1), A_k_cache, A_v_cache, A_wq, A_wo)
    h2 = h + _B_ref(_layernorm(h, axis=-1), B_w_r, B_w_gate, B_w_up, B_w_down)
    return h2
```

```python
import functools

import jax
import jax.numpy as jnp
import jax.experimental.pallas as pl
import jax.experimental.pallas.tpu as pltpu

_LN_EPS = 1e-5
_HQ = 32
_G = 2
_NB = 3
_M = 16
_FC = 6


def _layernorm(x):
    m = jnp.mean(x, axis=-1, keepdims=True)
    c = x - m
    v = jnp.mean(c * c, axis=-1, keepdims=True)
    return c / jnp.sqrt(v + _LN_EPS)


def _kernel(x_hbm, kt_hbm, vt_hbm, wq_hbm, wo_hbm, wr_hbm, wg_hbm, wu_hbm, wd_hbm,
            o_ref,
            x_buf, wr_buf, k_buf, v_buf, wq_buf, wo_buf, wg_buf, wu_buf, wd_buf, acc_ref,
            s_small, s_k, s_v, s_wq, s_wo, s_ffn,
            *, dh, sk, w):
    d = x_buf.shape[-1]
    gd = _G * dh
    nsteps = _HQ // _G
    f = wg_buf.shape[-1]
    fch = f // _FC

    def cp_k(j, slot):
        return pltpu.make_async_copy(
            kt_hbm.at[pl.ds(j * gd, gd), pl.ds(sk - w, w)], k_buf.at[slot], s_k.at[slot])

    def cp_v(j, slot):
        return pltpu.make_async_copy(
            vt_hbm.at[pl.ds(j * gd, gd), pl.ds(sk - w, w)], v_buf.at[slot], s_v.at[slot])

    def cp_wq(j):
        return pltpu.make_async_copy(
            wq_hbm.at[:, pl.ds(j * gd, gd)], wq_buf.at[j], s_wq.at[j])

    def cp_wo(j):
        return pltpu.make_async_copy(
            wo_hbm.at[pl.ds(j * gd, gd), :], wo_buf.at[j], s_wo.at[j])

    cp_x = pltpu.make_async_copy(x_hbm, x_buf, s_small.at[0])
    cp_wr = pltpu.make_async_copy(wr_hbm, wr_buf, s_small.at[1])
    cp_wg = pltpu.make_async_copy(wg_hbm, wg_buf, s_ffn.at[0])
    cp_wu = pltpu.make_async_copy(wu_hbm, wu_buf, s_ffn.at[1])

    def cp_wd(c):
        return pltpu.make_async_copy(
            wd_hbm.at[pl.ds(c * fch, fch), :], wd_buf.at[pl.ds(c * fch, fch), :], s_ffn.at[2 + c])

    def start_step(j, slot):
        cp_wq(j).start()
        cp_k(j, slot).start()
        cp_v(j, slot).start()
        cp_wo(j).start()

    cp_x.start()
    cp_wr.start()
    for j in range(_NB):
        start_step(j, j)

    cp_x.wait()
    x = x_buf[...].reshape(1, d).astype(jnp.float32)
    xn = jnp.broadcast_to(_layernorm(x), (_M, d)).astype(jnp.bfloat16)
    acc_ref[...] = jnp.zeros_like(acc_ref)

    row = jax.lax.broadcasted_iota(jnp.int32, (_M, gd), 0)
    col = jax.lax.broadcasted_iota(jnp.int32, (_M, gd), 1)
    diag = (col >= row * dh) & (col < (row + 1) * dh)
    scale = dh ** -0.5

    def step(j, carry):
        slot = j % _NB
        cp_wq(j).wait()
        q = jnp.dot(xn, wq_buf[j], preferred_element_type=jnp.float32)
        qbd = jnp.where(diag, q, 0.0).astype(jnp.bfloat16)
        cp_k(j, slot).wait()
        s = jnp.dot(qbd, k_buf[slot], preferred_element_type=jnp.float32) * scale
        m = jnp.max(s, axis=-1, keepdims=True)
        e = jnp.exp(s - m)
        l = jnp.sum(e, axis=-1, keepdims=True)
        p = (e / l).astype(jnp.bfloat16)
        cp_v(j, slot).wait()
        o = jax.lax.dot_general(p, v_buf[slot], (((1,), (1,)), ((), ())),
                                preferred_element_type=jnp.float32)
        obd = jnp.where(diag, o, 0.0).astype(jnp.bfloat16)
        cp_wo(j).wait()
        acc_ref[...] += jnp.dot(obd, wo_buf[j], preferred_element_type=jnp.float32)

        @pl.when(j + _NB < nsteps)
        def _():
            start_step(j + _NB, slot)

        @pl.when(j + _NB == nsteps)
        def _():
            cp_wg.start()
            cp_wu.start()
            for c in range(_FC):
                cp_wd(c).start()

        return carry

    jax.lax.fori_loop(0, nsteps, step, 0)

    attn = jnp.sum(acc_ref[...], axis=0, keepdims=True)
    h = x + attn
    hn = _layernorm(h)
    hb = jnp.broadcast_to(hn, (_M, d)).astype(jnp.bfloat16)
    cp_wr.wait()
    wr = wr_buf[...].reshape(1, d).astype(jnp.float32)
    r = jnp.sum(hn * wr, axis=-1, keepdims=True)
    gate = jax.nn.sigmoid(r)
    cp_wg.wait()
    g = jnp.dot(hb, wg_buf[...], preferred_element_type=jnp.float32)
    g = g * jax.nn.sigmoid(g)
    cp_wu.wait()
    u = jnp.dot(hb, wu_buf[...], preferred_element_type=jnp.float32)
    a = (g * u).astype(jnp.bfloat16)
    y = jnp.zeros((_M, d), jnp.float32)
    for c in range(_FC):
        cp_wd(c).wait()
        y = y + jnp.dot(a[:, c * fch:(c + 1) * fch], wd_buf[c * fch:(c + 1) * fch, :],
                        preferred_element_type=jnp.float32)
    out = h + hn + y[0:1, :] * gate
    o_ref[...] = out.reshape(o_ref.shape).astype(o_ref.dtype)


@jax.jit
def pallas_sequential_preLN__sliding_block_cached__moe_arch_mod__decode_kernel(
    A_x: jax.Array,
    A_k_cache: jax.Array,
    A_v_cache: jax.Array,
    A_wq: jax.Array,
    A_wo: jax.Array,
    B_x: jax.Array,
    B_w_r: jax.Array,
    B_w_gate: jax.Array,
    B_w_up: jax.Array,
    B_w_down: jax.Array,
):
    b, sq, d = A_x.shape
    _, hkv, sk, dh = A_k_cache.shape
    assert b == 1 and sq == 1 and hkv == _HQ
    w = min(4096, max(256, sk // 4))
    f = B_w_gate.shape[1]
    gd = _G * dh
    nsteps = _HQ // _G
    bf = jnp.bfloat16

    kt = jnp.swapaxes(A_k_cache, 2, 3).reshape(hkv * dh, sk)
    vt = jnp.swapaxes(A_v_cache, 2, 3).reshape(hkv * dh, sk)

    any_spec = pl.BlockSpec(memory_space=pl.ANY)
    return pl.pallas_call(
        functools.partial(_kernel, dh=dh, sk=sk, w=w),
        in_specs=[any_spec] * 9,
        out_specs=pl.BlockSpec(memory_space=pltpu.VMEM),
        out_shape=jax.ShapeDtypeStruct(A_x.shape, A_x.dtype),
        scratch_shapes=[
            pltpu.VMEM(A_x.shape, bf),
            pltpu.VMEM(B_w_r.shape, bf),
            pltpu.VMEM((_NB, gd, w), bf),
            pltpu.VMEM((_NB, gd, w), bf),
            pltpu.VMEM((nsteps, d, gd), bf),
            pltpu.VMEM((nsteps, gd, d), bf),
            pltpu.VMEM((d, f), bf),
            pltpu.VMEM((d, f), bf),
            pltpu.VMEM((f, d), bf),
            pltpu.VMEM((_M, d), jnp.float32),
            pltpu.SemaphoreType.DMA((2,)),
            pltpu.SemaphoreType.DMA((_NB,)),
            pltpu.SemaphoreType.DMA((_NB,)),
            pltpu.SemaphoreType.DMA((nsteps,)),
            pltpu.SemaphoreType.DMA((nsteps,)),
            pltpu.SemaphoreType.DMA((2 + _FC,)),
        ],
        compiler_params=pltpu.CompilerParams(vmem_limit_bytes=100 * 1024 * 1024),
    )(A_x, kt, vt, A_wq, A_wo, B_w_r, B_w_gate, B_w_up, B_w_down)
```

```python
import functools
import math

import jax
import jax.numpy as jnp
import jax.experimental.pallas as pl
import jax.experimental.pallas.tpu as pltpu

_LN_EPS = 1e-5
_HQ = 32
_G = 2
_M = 8
_BC = 512
_NR = 8
_LOOK = 7
_KV_SPLIT = (8, 56)
_GQ, _GO, _RW = 10, 8, 8
_LW = 32
_GATE_SPLIT = (8, 24)
_DOWN_SPLIT = (8, 56)


def _layernorm(x):
    m = jnp.mean(x, axis=-1, keepdims=True)
    c = x - m
    v = jnp.mean(c * c, axis=-1, keepdims=True)
    return c / jnp.sqrt(v + _LN_EPS)


def _hint(x, m):
    return x if isinstance(x, int) else pl.multiple_of(x, m)


def _row_splits(total, pat):
    hi, lo = pat
    assert total % (hi + lo) == 0
    out = []
    for r in range(0, total, hi + lo):
        out += [(r, hi), (r + hi, lo)]
    return out


def _start(el):
    el[0].start(priority=0)
    el[1].start(priority=1)


def _wait(el):
    el[0].wait()
    el[1].wait()


def _kernel(x_hbm, kt_hbm, vt_hbm, wq_hbm, wo_hbm, wr_hbm, wg_hbm, wu_hbm, wd_hbm,
            o_ref,
            x_buf, wr_buf, kv_buf, wq_buf, wo_buf, wg_buf, wu_buf, wd_buf,
            acc_ref, obd_ref, p_ref, q_ref,
            s_small, s_kv, s_w, s_down,
            *, dh, sk, w):
    d = x_buf.shape[-1]
    f = wg_buf.shape[-1]
    gd = _G * dh
    npair = _HQ // _G
    nb = w // _BC
    pb = 2 * nb
    bf = jnp.bfloat16
    assert pb % _NR == 0 and _LOOK < _NR and _LOOK <= nb

    hi, lo = _KV_SPLIT
    epb = gd // (hi + lo)
    kv_align = math.gcd(hi + lo, hi)

    def kv_el(pair, pos, c):
        src = kt_hbm if pos < nb else vt_hbm
        slot = pos % _NR
        out = []
        for r0, rows in ((c * (hi + lo), hi), (c * (hi + lo) + hi, lo)):
            out.append(pltpu.make_async_copy(
                src.at[pl.ds(_hint(pair * gd + r0, kv_align), rows), pl.ds(sk - w + (pos % nb) * _BC, _BC)],
                kv_buf.at[slot, pl.ds(r0, rows), :], s_kv.at[slot]))
        return out

    upq = d // _GQ // _RW
    nuq = npair * upq
    nuo = _HQ * dh // _GO // _RW
    ppg = _HQ * dh // _GO // gd

    def wq_el(u):
        pair = u // upq
        rows = pl.ds(_hint((u % upq) * _RW, _RW), _RW)
        return [pltpu.make_async_copy(
            wq_hbm.at[pl.ds(g0, gn), rows, pl.ds(_hint(pair * gd, 128), gd)],
            wq_buf.at[pair, pl.ds(g0, gn), rows, :], s_w.at[0]) for g0, gn in ((0, 1), (1, _GQ - 1))]

    def wo_el(u):
        rows = pl.ds(_hint(u * _RW, _RW), _RW)
        return [pltpu.make_async_copy(
            wo_hbm.at[pl.ds(g0, gn), rows, :], wo_buf.at[pl.ds(g0, gn), rows, :], s_w.at[1])
            for g0, gn in ((0, 1), (1, _GO - 1))]

    def row_els(src, dst, pat, sem_of):
        cps = [pltpu.make_async_copy(src.at[pl.ds(r0, n), :], dst.at[pl.ds(r0, n), :], sem_of(r0))
               for r0, n in _row_splits(src.shape[0], pat)]
        return [cps[i:i + 2] for i in range(0, len(cps), 2)]

    kslab = 128
    assert kslab % sum(_DOWN_SPLIT) == 0
    wg_els = row_els(wg_hbm, wg_buf, _GATE_SPLIT, lambda r: s_w.at[2])
    wu_els = row_els(wu_hbm, wu_buf, _GATE_SPLIT, lambda r: s_w.at[3])
    wd_els = row_els(wd_hbm, wd_buf, _DOWN_SPLIT, lambda r: s_down.at[r // kslab])
    ffn_els = wg_els + wu_els + wd_els
    ffn_started = [0]

    def start_next_ffn():
        if ffn_started[0] < len(ffn_els):
            _start(ffn_els[ffn_started[0]])
            ffn_started[0] += 1

    cp_x = pltpu.make_async_copy(x_hbm, x_buf, s_small.at[0])
    cp_wr = pltpu.make_async_copy(wr_hbm, wr_buf, s_small.at[1])

    row = jax.lax.broadcasted_iota(jnp.int32, (_M, gd), 0)
    col = jax.lax.broadcasted_iota(jnp.int32, (_M, gd), 1)
    diag = (col >= row * dh) & (col < (row + 1) * dh)
    scale = dh ** -0.5

    cp_x.start()
    for u in range(_LW):
        _start(wq_el(u))
    cp_wr.start()
    cp_x.wait()
    x = x_buf[...].reshape(1, d).astype(jnp.float32)
    xn = jnp.broadcast_to(_layernorm(x), (_M, d)).astype(bf)
    acc_ref[...] = jnp.zeros_like(acc_ref)
    obd_ref[...] = jnp.zeros_like(obd_ref)

    def wq_loop(u, carry):
        _wait(wq_el(u))
        _start(wq_el(u + _LW))
        return carry

    def wq_wo_loop(u, carry):
        _wait(wq_el(u))
        _start(wo_el(u + _LW - nuq))
        return carry

    jax.lax.fori_loop(0, nuq - _LW, wq_loop, 0)
    jax.lax.fori_loop(nuq - _LW, nuq, wq_wo_loop, 0)

    epq = (nuo - _LW) // npair

    def wo_loop(j, carry):
        for i in range(epq):
            u = j * epq + i
            _wait(wo_el(u))
            _start(wo_el(u + _LW))
        q = jnp.dot(xn, wq_buf[j].reshape(d, gd), preferred_element_type=jnp.float32)
        q_ref[j] = jnp.where(diag, q, 0.0).astype(bf)
        return carry

    jax.lax.fori_loop(0, npair, wo_loop, 0)
    for u in range(epq * npair, nuo - _LW):
        _wait(wo_el(u))
        _start(wo_el(u + _LW))
    n_first = _LOOK * epb
    k = 0
    for i, u in enumerate(range(nuo - _LW, nuo)):
        _wait(wo_el(u))
        while k < -(-(i + 1) * n_first // _LW):
            _start(kv_el(0, k // epb, k % epb))
            k += 1

    def out_proj(pair, c0, cn):
        wo = wo_buf.at[pair // ppg, pl.ds(_hint((pair % ppg) * gd, 16), gd), :]
        acc_ref[:, c0:c0 + cn] += jnp.dot(obd_ref[...], wo[:, c0:c0 + cn], preferred_element_type=jnp.float32)

    def pair_body(pair, last):
        s, m, l = [None] * nb, [None] * nb, [None] * nb

        def block_softmax(b):
            sb = s[b] * scale
            m[b] = jnp.max(sb, axis=-1, keepdims=True)
            e = jnp.exp(sb - m[b])
            l[b] = jnp.sum(e, axis=-1, keepdims=True)
            p_ref[b] = e.astype(bf)

        o = None
        for pos in range(pb):
            for c in range(epb):
                _wait(kv_el(pair, pos, c))
                if pos + _LOOK < pb:
                    _start(kv_el(pair, pos + _LOOK, c))
                elif not last:
                    _start(kv_el(pair + 1, pos + _LOOK - pb, c))
                else:
                    start_next_ffn()
            blk = kv_buf[pos % _NR]
            b = pos % nb
            if pos < nb:
                s[b] = jnp.dot(q_ref[pair], blk, preferred_element_type=jnp.float32)
                if b > 0:
                    block_softmax(b - 1)
                if pos < d // 128:
                    prev = max(pair - 1, 0) if last else jnp.maximum(pair - 1, 0)
                    out_proj(prev, pos * 128, 128)
            else:
                r = jax.lax.dot_general(p_ref[b], blk, (((1,), (1,)), ((), ())),
                                        preferred_element_type=jnp.float32)
                if b == 0:
                    block_softmax(nb - 1)
                    mx = functools.reduce(jnp.maximum, m)
                    fs = [jnp.exp(mb - mx) for mb in m]
                    linv = 1.0 / functools.reduce(jnp.add, [fb * lb for fb, lb in zip(fs, l)])
                r = r * fs[b]
                o = r if o is None else o + r
        obd_ref[...] = jnp.where(diag, o * linv, 0.0).astype(bf)

    def pair_loop(pair, carry):
        pair_body(pair, False)
        return carry

    jax.lax.fori_loop(0, npair - 1, pair_loop, 0)
    pair_body(npair - 1, True)

    out_proj(npair - 1, 0, d)
    x = x_buf[...].reshape(1, d).astype(jnp.float32)
    h = x + jnp.sum(acc_ref[...], axis=0, keepdims=True)
    hn = _layernorm(h)
    hb = jnp.broadcast_to(hn, (_M, d)).astype(bf)
    cp_wr.wait()
    wr = wr_buf[...].reshape(1, d).astype(jnp.float32)
    gate = jax.nn.sigmoid(jnp.sum(hn * wr, axis=-1, keepdims=True))

    def consume(els):
        for el in els:
            _wait(el)
            start_next_ffn()

    consume(wg_els)
    g = jnp.dot(hb, wg_buf[...], preferred_element_type=jnp.float32)
    g = g * jax.nn.sigmoid(g)
    consume(wu_els)
    u = jnp.dot(hb, wu_buf[...], preferred_element_type=jnp.float32)
    a = (g * u).astype(bf)
    y = jnp.zeros((_M, d), jnp.float32)
    eps = kslab // sum(_DOWN_SPLIT)
    for i in range(f // kslab):
        consume(wd_els[i * eps:(i + 1) * eps])
        y = y + jnp.dot(a[:, i * kslab:(i + 1) * kslab], wd_buf[i * kslab:(i + 1) * kslab, :],
                        preferred_element_type=jnp.float32)
    assert ffn_started[0] == len(ffn_els)
    out = h + hn + y[0:1, :] * gate
    o_ref[...] = out.reshape(o_ref.shape).astype(o_ref.dtype)


def _compiler_params():
    kw = dict(vmem_limit_bytes=64 * 1024 * 1024)
    if hasattr(pltpu.CompilerParams, "disable_semaphore_checks"):
        kw["disable_semaphore_checks"] = True
    return pltpu.CompilerParams(**kw)


@jax.jit
def pallas_sequential_preLN__sliding_block_cached__moe_arch_mod__decode_kernel(
    A_x: jax.Array,
    A_k_cache: jax.Array,
    A_v_cache: jax.Array,
    A_wq: jax.Array,
    A_wo: jax.Array,
    B_x: jax.Array,
    B_w_r: jax.Array,
    B_w_gate: jax.Array,
    B_w_up: jax.Array,
    B_w_down: jax.Array,
):
    b, sq, d = A_x.shape
    _, hkv, sk, dh = A_k_cache.shape
    assert b == 1 and sq == 1 and hkv == _HQ
    w = min(4096, max(256, sk // 4))
    f = B_w_gate.shape[1]
    gd = _G * dh
    npair = _HQ // _G
    bf = jnp.bfloat16

    kt = jnp.swapaxes(A_k_cache, 2, 3).reshape(hkv * dh, sk)
    vt = jnp.swapaxes(A_v_cache, 2, 3).reshape(hkv * dh, sk)
    wq3 = A_wq.reshape(_GQ, d // _GQ, hkv * dh)
    wo3 = A_wo.reshape(_GO, hkv * dh // _GO, d)

    any_spec = pl.BlockSpec(memory_space=pl.ANY)
    return pl.pallas_call(
        functools.partial(_kernel, dh=dh, sk=sk, w=w),
        in_specs=[any_spec] * 9,
        out_specs=pl.BlockSpec(memory_space=pltpu.VMEM),
        out_shape=jax.ShapeDtypeStruct(A_x.shape, A_x.dtype),
        scratch_shapes=[
            pltpu.VMEM(A_x.shape, bf),
            pltpu.VMEM(B_w_r.shape, bf),
            pltpu.VMEM((_NR, gd, _BC), bf),
            pltpu.VMEM((npair, _GQ, d // _GQ, gd), bf),
            pltpu.VMEM((_GO, hkv * dh // _GO, d), bf),
            pltpu.VMEM((d, f), bf),
            pltpu.VMEM((d, f), bf),
            pltpu.VMEM((f, d), bf),
            pltpu.VMEM((_M, d), jnp.float32),
            pltpu.VMEM((_M, gd), bf),
            pltpu.VMEM((w // _BC, _M, _BC), bf),
            pltpu.VMEM((npair, _M, gd), bf),
            pltpu.SemaphoreType.DMA((2,)),
            pltpu.SemaphoreType.DMA((_NR,)),
            pltpu.SemaphoreType.DMA((4,)),
            pltpu.SemaphoreType.DMA((f // 128,)),
        ],
        compiler_params=_compiler_params(),
    )(A_x, kt, vt, wq3, wo3, B_w_r, B_w_gate, B_w_up, B_w_down)
```

```python
import functools
import math

import jax
import jax.numpy as jnp
import jax.experimental.pallas as pl
import jax.experimental.pallas.tpu as pltpu

_LN_EPS = 1e-5
_HQ = 32
_G = 2
_M = 8
_BC = 1024
_NR = 8
_LOOK = 5
_KV_SPLIT = (8, 16)
_GQ, _GO, _RW = 10, 8, 8
_LW = 32
_GATE_SPLIT = (8, 24)
_DOWN_SPLIT = (8, 56)


def _layernorm(x):
    m = jnp.mean(x, axis=-1, keepdims=True)
    c = x - m
    v = jnp.mean(c * c, axis=-1, keepdims=True)
    return c / jnp.sqrt(v + _LN_EPS)


def _hint(x, m):
    return x if isinstance(x, int) else pl.multiple_of(x, m)


def _row_splits(total, pat):
    hi, lo = pat
    assert total % (hi + lo) == 0
    out = []
    for r in range(0, total, hi + lo):
        out += [(r, hi), (r + hi, lo)]
    return out


def _start(el):
    el[0].start(priority=0)
    el[1].start(priority=1)


def _wait(el):
    el[0].wait()
    el[1].wait()


def _kernel(x_hbm, kt_hbm, vt_hbm, wq_hbm, wo_hbm, wr_hbm, wg_hbm, wu_hbm, wd_hbm,
            o_ref,
            x_buf, wr_buf, kv_buf, wq_buf, wo_buf, wg_buf, wu_buf, wd_buf,
            acc_ref, obd_ref, p_ref, q_ref,
            s_small, s_kv, s_w, s_down,
            *, dh, sk, w):
    d = x_buf.shape[-1]
    f = wg_buf.shape[-1]
    gd = _G * dh
    npair = _HQ // _G
    nb = w // _BC
    pb = 2 * nb
    bf = jnp.bfloat16
    assert pb % _NR == 0 and _LOOK < _NR and gd % sum(_KV_SPLIT) == 0

    hi, lo = _KV_SPLIT
    epb = gd // (hi + lo)
    kv_align = math.gcd(hi + lo, hi)

    def kv_el(pair, pos, c):
        src = kt_hbm if pos < nb else vt_hbm
        slot = pos % _NR
        out = []
        for r0, rows in ((c * (hi + lo), hi), (c * (hi + lo) + hi, lo)):
            out.append(pltpu.make_async_copy(
                src.at[pl.ds(_hint(pair * gd + r0, kv_align), rows), pl.ds(sk - w + (pos % nb) * _BC, _BC)],
                kv_buf.at[slot, pl.ds(r0, rows), :], s_kv.at[slot]))
        return out

    upq = d // _GQ // _RW
    nuq = npair * upq
    nuo = _HQ * dh // _GO // _RW
    ppg = _HQ * dh // _GO // gd

    def wq_el(u):
        pair = u // upq
        rows = pl.ds(_hint((u % upq) * _RW, _RW), _RW)
        return [pltpu.make_async_copy(
            wq_hbm.at[pl.ds(g0, gn), rows, pl.ds(_hint(pair * gd, 128), gd)],
            wq_buf.at[pair, pl.ds(g0, gn), rows, :], s_w.at[0]) for g0, gn in ((0, 1), (1, _GQ - 1))]

    def wo_el(u):
        rows = pl.ds(_hint(u * _RW, _RW), _RW)
        return [pltpu.make_async_copy(
            wo_hbm.at[pl.ds(g0, gn), rows, :], wo_buf.at[pl.ds(g0, gn), rows, :], s_w.at[1])
            for g0, gn in ((0, 1), (1, _GO - 1))]

    def row_els(src, dst, pat, sem_of):
        cps = [pltpu.make_async_copy(src.at[pl.ds(r0, n), :], dst.at[pl.ds(r0, n), :], sem_of(r0))
               for r0, n in _row_splits(src.shape[0], pat)]
        return [cps[i:i + 2] for i in range(0, len(cps), 2)]

    kslab = 128
    assert kslab % sum(_DOWN_SPLIT) == 0
    wg_els = row_els(wg_hbm, wg_buf, _GATE_SPLIT, lambda r: s_w.at[2])
    wu_els = row_els(wu_hbm, wu_buf, _GATE_SPLIT, lambda r: s_w.at[3])
    wd_els = row_els(wd_hbm, wd_buf, _DOWN_SPLIT, lambda r: s_down.at[r // kslab])
    ffn_els = wg_els + wu_els + wd_els
    ffn_started = [0]

    def start_next_ffn():
        if ffn_started[0] < len(ffn_els):
            _start(ffn_els[ffn_started[0]])
            ffn_started[0] += 1

    cp_x = pltpu.make_async_copy(x_hbm, x_buf, s_small.at[0])
    cp_wr = pltpu.make_async_copy(wr_hbm, wr_buf, s_small.at[1])

    row = jax.lax.broadcasted_iota(jnp.int32, (_M, gd), 0)
    col = jax.lax.broadcasted_iota(jnp.int32, (_M, gd), 1)
    diag = (col >= row * dh) & (col < (row + 1) * dh)
    scale = dh ** -0.5

    cp_x.start()
    for u in range(_LW):
        _start(wq_el(u))
    cp_wr.start()
    cp_x.wait()
    x = x_buf[...].reshape(1, d).astype(jnp.float32)
    xn = jnp.broadcast_to(_layernorm(x), (_M, d)).astype(bf)
    acc_ref[...] = jnp.zeros_like(acc_ref)
    obd_ref[...] = jnp.zeros_like(obd_ref)

    def wq_loop(u, carry):
        _wait(wq_el(u))
        _start(wq_el(u + _LW))
        return carry

    def wq_wo_loop(u, carry):
        _wait(wq_el(u))
        _start(wo_el(u + _LW - nuq))
        return carry

    jax.lax.fori_loop(0, nuq - _LW, wq_loop, 0)
    jax.lax.fori_loop(nuq - _LW, nuq, wq_wo_loop, 0)

    epq = (nuo - _LW) // npair

    def wo_loop(j, carry):
        for i in range(epq):
            u = j * epq + i
            _wait(wo_el(u))
            _start(wo_el(u + _LW))
        q = jnp.dot(xn, wq_buf[j].reshape(d, gd), preferred_element_type=jnp.float32)
        q_ref[j] = jnp.where(diag, q, 0.0).astype(bf)
        return carry

    jax.lax.fori_loop(0, npair, wo_loop, 0)
    for u in range(epq * npair, nuo - _LW):
        _wait(wo_el(u))
        _start(wo_el(u + _LW))
    n_first = _LOOK * epb
    k = 0
    for i, u in enumerate(range(nuo - _LW, nuo)):
        _wait(wo_el(u))
        while k < -(-(i + 1) * n_first // _LW):
            _start(kv_el(0, k // epb, k % epb))
            k += 1

    def out_proj(pair, c0, cn):
        wo = wo_buf.at[pair // ppg, pl.ds(_hint((pair % ppg) * gd, 16), gd), :]
        acc_ref[:, c0:c0 + cn] += jnp.dot(obd_ref[...], wo[:, c0:c0 + cn], preferred_element_type=jnp.float32)

    def pair_body(pair, last):
        s, m, l = [None] * nb, [None] * nb, [None] * nb

        def block_softmax(b):
            sb = s[b] * scale
            m[b] = jnp.max(sb, axis=-1, keepdims=True)
            e = jnp.exp(sb - m[b])
            l[b] = jnp.sum(e, axis=-1, keepdims=True)
            p_ref[b] = e.astype(bf)

        o = None
        for pos in range(pb):
            for c in range(epb):
                _wait(kv_el(pair, pos, c))
                if pos + _LOOK < pb:
                    _start(kv_el(pair, pos + _LOOK, c))
                elif not last:
                    _start(kv_el(pair + 1, pos + _LOOK - pb, c))
                else:
                    start_next_ffn()
            blk = kv_buf[pos % _NR]
            b = pos % nb
            if pos < d // 128:
                prev = max(pair - 1, 0) if last else jnp.maximum(pair - 1, 0)
                out_proj(prev, pos * 128, 128)
            if pos < nb:
                s[b] = jnp.dot(q_ref[pair], blk, preferred_element_type=jnp.float32)
                if b > 0:
                    block_softmax(b - 1)
            else:
                r = jax.lax.dot_general(p_ref[b], blk, (((1,), (1,)), ((), ())),
                                        preferred_element_type=jnp.float32)
                if b == 0:
                    block_softmax(nb - 1)
                    mx = functools.reduce(jnp.maximum, m)
                    fs = [jnp.exp(mb - mx) for mb in m]
                    linv = 1.0 / functools.reduce(jnp.add, [fb * lb for fb, lb in zip(fs, l)])
                r = r * fs[b]
                o = r if o is None else o + r
        obd_ref[...] = jnp.where(diag, o * linv, 0.0).astype(bf)

    def pair_loop(pair, carry):
        pair_body(pair, False)
        return carry

    jax.lax.fori_loop(0, npair - 1, pair_loop, 0)
    pair_body(npair - 1, True)

    out_proj(npair - 1, 0, d)
    x = x_buf[...].reshape(1, d).astype(jnp.float32)
    h = x + jnp.sum(acc_ref[...], axis=0, keepdims=True)
    hn = _layernorm(h)
    hb = jnp.broadcast_to(hn, (_M, d)).astype(bf)
    cp_wr.wait()
    wr = wr_buf[...].reshape(1, d).astype(jnp.float32)
    gate = jax.nn.sigmoid(jnp.sum(hn * wr, axis=-1, keepdims=True))

    def consume(els):
        for el in els:
            _wait(el)
            start_next_ffn()

    consume(wg_els)
    g = jnp.dot(hb, wg_buf[...], preferred_element_type=jnp.float32)
    g = g * jax.nn.sigmoid(g)
    consume(wu_els)
    u = jnp.dot(hb, wu_buf[...], preferred_element_type=jnp.float32)
    a = (g * u).astype(bf)
    y = jnp.zeros((_M, d), jnp.float32)
    eps = kslab // sum(_DOWN_SPLIT)
    for i in range(f // kslab):
        consume(wd_els[i * eps:(i + 1) * eps])
        y = y + jnp.dot(a[:, i * kslab:(i + 1) * kslab], wd_buf[i * kslab:(i + 1) * kslab, :],
                        preferred_element_type=jnp.float32)
    assert ffn_started[0] == len(ffn_els)
    out = h + hn + y[0:1, :] * gate
    o_ref[...] = out.reshape(o_ref.shape).astype(o_ref.dtype)


def _compiler_params():
    kw = dict(vmem_limit_bytes=64 * 1024 * 1024)
    if hasattr(pltpu.CompilerParams, "disable_semaphore_checks"):
        kw["disable_semaphore_checks"] = True
    return pltpu.CompilerParams(**kw)


@jax.jit
def pallas_sequential_preLN__sliding_block_cached__moe_arch_mod__decode_kernel(
    A_x: jax.Array,
    A_k_cache: jax.Array,
    A_v_cache: jax.Array,
    A_wq: jax.Array,
    A_wo: jax.Array,
    B_x: jax.Array,
    B_w_r: jax.Array,
    B_w_gate: jax.Array,
    B_w_up: jax.Array,
    B_w_down: jax.Array,
):
    b, sq, d = A_x.shape
    _, hkv, sk, dh = A_k_cache.shape
    assert b == 1 and sq == 1 and hkv == _HQ
    w = min(4096, max(256, sk // 4))
    f = B_w_gate.shape[1]
    gd = _G * dh
    npair = _HQ // _G
    bf = jnp.bfloat16

    kt = jnp.swapaxes(A_k_cache, 2, 3).reshape(hkv * dh, sk)
    vt = jnp.swapaxes(A_v_cache, 2, 3).reshape(hkv * dh, sk)
    wq3 = A_wq.reshape(_GQ, d // _GQ, hkv * dh)
    wo3 = A_wo.reshape(_GO, hkv * dh // _GO, d)

    any_spec = pl.BlockSpec(memory_space=pl.ANY)
    return pl.pallas_call(
        functools.partial(_kernel, dh=dh, sk=sk, w=w),
        in_specs=[any_spec] * 9,
        out_specs=pl.BlockSpec(memory_space=pltpu.VMEM),
        out_shape=jax.ShapeDtypeStruct(A_x.shape, A_x.dtype),
        scratch_shapes=[
            pltpu.VMEM(A_x.shape, bf),
            pltpu.VMEM(B_w_r.shape, bf),
            pltpu.VMEM((_NR, gd, _BC), bf),
            pltpu.VMEM((npair, _GQ, d // _GQ, gd), bf),
            pltpu.VMEM((_GO, hkv * dh // _GO, d), bf),
            pltpu.VMEM((d, f), bf),
            pltpu.VMEM((d, f), bf),
            pltpu.VMEM((f, d), bf),
            pltpu.VMEM((_M, d), jnp.float32),
            pltpu.VMEM((_M, gd), bf),
            pltpu.VMEM((w // _BC, _M, _BC), bf),
            pltpu.VMEM((npair, _M, gd), bf),
            pltpu.SemaphoreType.DMA((2,)),
            pltpu.SemaphoreType.DMA((_NR,)),
            pltpu.SemaphoreType.DMA((4,)),
            pltpu.SemaphoreType.DMA((f // 128,)),
        ],
        compiler_params=_compiler_params(),
    )(A_x, kt, vt, wq3, wo3, B_w_r, B_w_gate, B_w_up, B_w_down)
```

```python
import functools

import jax
import jax.numpy as jnp
import jax.experimental.pallas as pl
import jax.experimental.pallas.tpu as pltpu

_LN_EPS = 1e-5
_HQ = 32
_G = 2
_M = 8
_BC = 1024
_NR = 8
_LOOK = 5
_KV_PRIO = (0, 1, 1, 1)
_GQ, _GO, _RW = 10, 8, 8
_LW = 32
_GATE_SPLIT = (8, 24)
_DOWN_SPLIT = (8, 56)


def _layernorm(x):
    m = jnp.mean(x, axis=-1, keepdims=True)
    c = x - m
    v = jnp.mean(c * c, axis=-1, keepdims=True)
    return c / jnp.sqrt(v + _LN_EPS)


def _hint(x, m):
    return x if isinstance(x, int) else pl.multiple_of(x, m)


def _row_splits(total, pat):
    hi, lo = pat
    assert total % (hi + lo) == 0
    out = []
    for r in range(0, total, hi + lo):
        out += [(r, hi), (r + hi, lo)]
    return out


def _start(el):
    for cp, prio in el:
        cp.start(priority=prio)


def _wait(el):
    for cp, _ in el:
        cp.wait()


def _kernel(x_hbm, kt_hbm, vt_hbm, wq_hbm, wo_hbm, wr_hbm, wg_hbm, wu_hbm, wd_hbm,
            o_ref,
            x_buf, wr_buf, kv_buf, wq_buf, wo_buf, wg_buf, wu_buf, wd_buf,
            acc_ref, obd_ref, p_ref, q_ref,
            s_small, s_kv, s_w, s_down,
            *, dh, sk, w):
    d = x_buf.shape[-1]
    f = wg_buf.shape[-1]
    gd = _G * dh
    npair = _HQ // _G
    nb = w // _BC
    pb = 2 * nb
    bf = jnp.bfloat16
    assert pb % _NR == 0 and _LOOK < _NR and gd % (8 * len(_KV_PRIO)) == 0

    erows = 8 * len(_KV_PRIO)
    epb = gd // erows

    def kv_el(pair, pos, c):
        src = kt_hbm if pos < nb else vt_hbm
        slot = pos % _NR
        out = []
        for i, prio in enumerate(_KV_PRIO):
            r0 = c * erows + 8 * i
            out.append((pltpu.make_async_copy(
                src.at[pl.ds(_hint(pair * gd + r0, 8), 8), pl.ds(sk - w + (pos % nb) * _BC, _BC)],
                kv_buf.at[slot, pl.ds(r0, 8), :], s_kv.at[slot]), prio))
        return out

    upq = d // _GQ // _RW
    nuq = npair * upq
    nuo = _HQ * dh // _GO // _RW
    ppg = _HQ * dh // _GO // gd

    def wq_el(u):
        pair = u // upq
        rows = pl.ds(_hint((u % upq) * _RW, _RW), _RW)
        return [(pltpu.make_async_copy(
            wq_hbm.at[pl.ds(g0, gn), rows, pl.ds(_hint(pair * gd, 128), gd)],
            wq_buf.at[pair, pl.ds(g0, gn), rows, :], s_w.at[0]), prio)
            for g0, gn, prio in ((0, 1, 0), (1, _GQ - 1, 1))]

    def wo_el(u):
        rows = pl.ds(_hint(u * _RW, _RW), _RW)
        return [(pltpu.make_async_copy(
            wo_hbm.at[pl.ds(g0, gn), rows, :], wo_buf.at[pl.ds(g0, gn), rows, :], s_w.at[1]), prio)
            for g0, gn, prio in ((0, 1, 0), (1, _GO - 1, 1))]

    def row_els(src, dst, pat, sem_of):
        cps = [pltpu.make_async_copy(src.at[pl.ds(r0, n), :], dst.at[pl.ds(r0, n), :], sem_of(r0))
               for r0, n in _row_splits(src.shape[0], pat)]
        return [[(cps[i], 0), (cps[i + 1], 1)] for i in range(0, len(cps), 2)]

    kslab = 128
    assert kslab % sum(_DOWN_SPLIT) == 0
    wg_els = row_els(wg_hbm, wg_buf, _GATE_SPLIT, lambda r: s_w.at[2])
    wu_els = row_els(wu_hbm, wu_buf, _GATE_SPLIT, lambda r: s_w.at[3])
    wd_els = row_els(wd_hbm, wd_buf, _DOWN_SPLIT, lambda r: s_down.at[r // kslab])
    ffn_els = wg_els + wu_els + wd_els
    ffn_started = [0]

    def start_next_ffn():
        if ffn_started[0] < len(ffn_els):
            _start(ffn_els[ffn_started[0]])
            ffn_started[0] += 1

    cp_x = pltpu.make_async_copy(x_hbm, x_buf, s_small.at[0])
    cp_wr = pltpu.make_async_copy(wr_hbm, wr_buf, s_small.at[1])

    row = jax.lax.broadcasted_iota(jnp.int32, (_M, gd), 0)
    col = jax.lax.broadcasted_iota(jnp.int32, (_M, gd), 1)
    diag = (col >= row * dh) & (col < (row + 1) * dh)
    scale = dh ** -0.5

    cp_x.start()
    for u in range(_LW):
        _start(wq_el(u))
    cp_wr.start()
    cp_x.wait()
    x = x_buf[...].reshape(1, d).astype(jnp.float32)
    xn = jnp.broadcast_to(_layernorm(x), (_M, d)).astype(bf)
    acc_ref[...] = jnp.zeros_like(acc_ref)
    obd_ref[...] = jnp.zeros_like(obd_ref)

    def wq_loop(u, carry):
        _wait(wq_el(u))
        _start(wq_el(u + _LW))
        return carry

    def wq_wo_loop(u, carry):
        _wait(wq_el(u))
        _start(wo_el(u + _LW - nuq))
        return carry

    jax.lax.fori_loop(0, nuq - _LW, wq_loop, 0)
    jax.lax.fori_loop(nuq - _LW, nuq, wq_wo_loop, 0)

    epq = (nuo - _LW) // npair

    def wo_loop(j, carry):
        for i in range(epq):
            u = j * epq + i
            _wait(wo_el(u))
            _start(wo_el(u + _LW))
        q = jnp.dot(xn, wq_buf[j].reshape(d, gd), preferred_element_type=jnp.float32)
        q_ref[j] = jnp.where(diag, q, 0.0).astype(bf)
        return carry

    jax.lax.fori_loop(0, npair, wo_loop, 0)
    for u in range(epq * npair, nuo - _LW):
        _wait(wo_el(u))
        _start(wo_el(u + _LW))
    n_first = _LOOK * epb
    k = 0
    for i, u in enumerate(range(nuo - _LW, nuo)):
        _wait(wo_el(u))
        while k < -(-(i + 1) * n_first // _LW):
            _start(kv_el(0, k // epb, k % epb))
            k += 1

    def out_proj(pair, c0, cn):
        wo = wo_buf.at[pair // ppg, pl.ds(_hint((pair % ppg) * gd, 16), gd), :]
        acc_ref[:, c0:c0 + cn] += jnp.dot(obd_ref[...], wo[:, c0:c0 + cn], preferred_element_type=jnp.float32)

    def pair_body(pair, last):
        s, m, l = [None] * nb, [None] * nb, [None] * nb

        def block_softmax(b):
            sb = s[b] * scale
            m[b] = jnp.max(sb, axis=-1, keepdims=True)
            e = jnp.exp(sb - m[b])
            l[b] = jnp.sum(e, axis=-1, keepdims=True)
            p_ref[b] = e.astype(bf)

        o = None
        for pos in range(pb):
            for c in range(epb):
                _wait(kv_el(pair, pos, c))
                if pos + _LOOK < pb:
                    _start(kv_el(pair, pos + _LOOK, c))
                elif not last:
                    _start(kv_el(pair + 1, pos + _LOOK - pb, c))
                else:
                    start_next_ffn()
            blk = kv_buf[pos % _NR]
            b = pos % nb
            if pos < d // 128:
                prev = max(pair - 1, 0) if last else jnp.maximum(pair - 1, 0)
                out_proj(prev, pos * 128, 128)
            if pos < nb:
                s[b] = jnp.dot(q_ref[pair], blk, preferred_element_type=jnp.float32)
                if b > 0:
                    block_softmax(b - 1)
            else:
                r = jax.lax.dot_general(p_ref[b], blk, (((1,), (1,)), ((), ())),
                                        preferred_element_type=jnp.float32)
                if b == 0:
                    block_softmax(nb - 1)
                    mx = functools.reduce(jnp.maximum, m)
                    fs = [jnp.exp(mb - mx) for mb in m]
                    linv = 1.0 / functools.reduce(jnp.add, [fb * lb for fb, lb in zip(fs, l)])
                r = r * fs[b]
                o = r if o is None else o + r
        obd_ref[...] = jnp.where(diag, o * linv, 0.0).astype(bf)

    def pair_loop(pair, carry):
        pair_body(pair, False)
        return carry

    jax.lax.fori_loop(0, npair - 1, pair_loop, 0)
    pair_body(npair - 1, True)

    out_proj(npair - 1, 0, d)
    x = x_buf[...].reshape(1, d).astype(jnp.float32)
    h = x + jnp.sum(acc_ref[...], axis=0, keepdims=True)
    hn = _layernorm(h)
    hb = jnp.broadcast_to(hn, (_M, d)).astype(bf)
    cp_wr.wait()
    wr = wr_buf[...].reshape(1, d).astype(jnp.float32)
    gate = jax.nn.sigmoid(jnp.sum(hn * wr, axis=-1, keepdims=True))

    def consume(els):
        for el in els:
            _wait(el)
            start_next_ffn()

    consume(wg_els)
    g = jnp.dot(hb, wg_buf[...], preferred_element_type=jnp.float32)
    g = g * jax.nn.sigmoid(g)
    consume(wu_els)
    u = jnp.dot(hb, wu_buf[...], preferred_element_type=jnp.float32)
    a = (g * u).astype(bf)
    y = jnp.zeros((_M, d), jnp.float32)
    eps = kslab // sum(_DOWN_SPLIT)
    for i in range(f // kslab):
        consume(wd_els[i * eps:(i + 1) * eps])
        y = y + jnp.dot(a[:, i * kslab:(i + 1) * kslab], wd_buf[i * kslab:(i + 1) * kslab, :],
                        preferred_element_type=jnp.float32)
    assert ffn_started[0] == len(ffn_els)
    out = h + hn + y[0:1, :] * gate
    o_ref[...] = out.reshape(o_ref.shape).astype(o_ref.dtype)


def _compiler_params():
    kw = dict(vmem_limit_bytes=64 * 1024 * 1024)
    if hasattr(pltpu.CompilerParams, "disable_semaphore_checks"):
        kw["disable_semaphore_checks"] = True
    return pltpu.CompilerParams(**kw)


@jax.jit
def pallas_sequential_preLN__sliding_block_cached__moe_arch_mod__decode_kernel(
    A_x: jax.Array,
    A_k_cache: jax.Array,
    A_v_cache: jax.Array,
    A_wq: jax.Array,
    A_wo: jax.Array,
    B_x: jax.Array,
    B_w_r: jax.Array,
    B_w_gate: jax.Array,
    B_w_up: jax.Array,
    B_w_down: jax.Array,
):
    b, sq, d = A_x.shape
    _, hkv, sk, dh = A_k_cache.shape
    assert b == 1 and sq == 1 and hkv == _HQ
    w = min(4096, max(256, sk // 4))
    f = B_w_gate.shape[1]
    gd = _G * dh
    npair = _HQ // _G
    bf = jnp.bfloat16

    kt = jnp.swapaxes(A_k_cache, 2, 3).reshape(hkv * dh, sk)
    vt = jnp.swapaxes(A_v_cache, 2, 3).reshape(hkv * dh, sk)
    wq3 = A_wq.reshape(_GQ, d // _GQ, hkv * dh)
    wo3 = A_wo.reshape(_GO, hkv * dh // _GO, d)

    any_spec = pl.BlockSpec(memory_space=pl.ANY)
    return pl.pallas_call(
        functools.partial(_kernel, dh=dh, sk=sk, w=w),
        in_specs=[any_spec] * 9,
        out_specs=pl.BlockSpec(memory_space=pltpu.VMEM),
        out_shape=jax.ShapeDtypeStruct(A_x.shape, A_x.dtype),
        scratch_shapes=[
            pltpu.VMEM(A_x.shape, bf),
            pltpu.VMEM(B_w_r.shape, bf),
            pltpu.VMEM((_NR, gd, _BC), bf),
            pltpu.VMEM((npair, _GQ, d // _GQ, gd), bf),
            pltpu.VMEM((_GO, hkv * dh // _GO, d), bf),
            pltpu.VMEM((d, f), bf),
            pltpu.VMEM((d, f), bf),
            pltpu.VMEM((f, d), bf),
            pltpu.VMEM((_M, d), jnp.float32),
            pltpu.VMEM((_M, gd), bf),
            pltpu.VMEM((w // _BC, _M, _BC), bf),
            pltpu.VMEM((npair, _M, gd), bf),
            pltpu.SemaphoreType.DMA((2,)),
            pltpu.SemaphoreType.DMA((_NR,)),
            pltpu.SemaphoreType.DMA((4,)),
            pltpu.SemaphoreType.DMA((f // 128,)),
        ],
        compiler_params=_compiler_params(),
    )(A_x, kt, vt, wq3, wo3, B_w_r, B_w_gate, B_w_up, B_w_down)
```

```python
import functools

import jax
import jax.numpy as jnp
import jax.experimental.pallas as pl
import jax.experimental.pallas.tpu as pltpu

_LN_EPS = 1e-5
_HQ = 32
_G = 2
_M = 8
_BC = 1024
_NR = 8
_LOOK = 5
_KV_PRIO = (0, 1, 1, 1)
_GQ, _GO, _RW = 10, 8, 8
_LW = 32
_GATE_SPLIT = (8, 24)
_DOWN_SPLIT = (8, 56)


def _layernorm(x):
    m = jnp.mean(x, axis=-1, keepdims=True)
    c = x - m
    v = jnp.mean(c * c, axis=-1, keepdims=True)
    return c / jnp.sqrt(v + _LN_EPS)


def _hint(x, m):
    return x if isinstance(x, int) else pl.multiple_of(x, m)


def _row_splits(total, pat):
    hi, lo = pat
    assert total % (hi + lo) == 0
    out = []
    for r in range(0, total, hi + lo):
        out += [(r, hi), (r + hi, lo)]
    return out


def _start(el):
    for cp, prio in el:
        cp.start(priority=prio)


def _wait(el):
    for cp, _ in el:
        cp.wait()


def _kernel(x_hbm, kt_hbm, vt_hbm, wq_hbm, wo_hbm, wr_hbm, wg_hbm, wu_hbm, wd_hbm,
            o_ref,
            x_buf, wr_buf, kv_buf, wq_buf, wo_buf, wg_buf, wu_buf, wd_buf,
            acc_ref, obd_ref, p_ref, q_ref,
            s_small, s_kv, s_w, s_down,
            *, dh, sk, w):
    d = x_buf.shape[-1]
    f = wg_buf.shape[-1]
    gd = _G * dh
    npair = _HQ // _G
    nb = w // _BC
    pb = 2 * nb
    bf = jnp.bfloat16
    assert pb % _NR == 0 and _LOOK < _NR and gd % (8 * len(_KV_PRIO)) == 0

    erows = 8 * len(_KV_PRIO)
    epb = gd // erows

    def kv_el(pair, pos, c):
        src = kt_hbm if pos < nb else vt_hbm
        slot = pos % _NR
        out = []
        for i, prio in enumerate(_KV_PRIO):
            r0 = c * erows + 8 * i
            out.append((pltpu.make_async_copy(
                src.at[pl.ds(_hint(pair * gd + r0, 8), 8), pl.ds(sk - w + (pos % nb) * _BC, _BC)],
                kv_buf.at[slot, pl.ds(r0, 8), :], s_kv.at[slot]), prio))
        return out

    upq = d // _GQ // _RW
    nuq = npair * upq
    nuo = _HQ * dh // _GO // _RW
    ppg = _HQ * dh // _GO // gd

    def wq_el(u):
        pair = u // upq
        rows = pl.ds(_hint((u % upq) * _RW, _RW), _RW)
        return [(pltpu.make_async_copy(
            wq_hbm.at[pl.ds(g0, gn), rows, pl.ds(_hint(pair * gd, 128), gd)],
            wq_buf.at[pair, pl.ds(g0, gn), rows, :], s_w.at[0]), prio)
            for g0, gn, prio in ((0, 1, 0), (1, _GQ - 1, 1))]

    def wo_el(u):
        rows = pl.ds(_hint(u * _RW, _RW), _RW)
        return [(pltpu.make_async_copy(
            wo_hbm.at[pl.ds(g0, gn), rows, :], wo_buf.at[pl.ds(g0, gn), rows, :], s_w.at[1]), prio)
            for g0, gn, prio in ((0, 1, 0), (1, _GO - 1, 1))]

    def row_els(src, dst, pat, sem_of):
        cps = [pltpu.make_async_copy(src.at[pl.ds(r0, n), :], dst.at[pl.ds(r0, n), :], sem_of(r0))
               for r0, n in _row_splits(src.shape[0], pat)]
        return [[(cps[i], 0), (cps[i + 1], 1)] for i in range(0, len(cps), 2)]

    kslab = 128
    assert kslab % sum(_DOWN_SPLIT) == 0
    wg_els = row_els(wg_hbm, wg_buf, _GATE_SPLIT, lambda r: s_w.at[2])
    wu_els = row_els(wu_hbm, wu_buf, _GATE_SPLIT, lambda r: s_w.at[3])
    wd_els = row_els(wd_hbm, wd_buf, _DOWN_SPLIT, lambda r: s_down.at[r // kslab])
    ffn_els = wg_els + wu_els + wd_els
    n_ffn_early = min(_LOOK * epb, len(ffn_els))

    cp_x = pltpu.make_async_copy(x_hbm, x_buf, s_small.at[0])
    cp_wr = pltpu.make_async_copy(wr_hbm, wr_buf, s_small.at[1])

    row = jax.lax.broadcasted_iota(jnp.int32, (_M, gd), 0)
    col = jax.lax.broadcasted_iota(jnp.int32, (_M, gd), 1)
    diag = (col >= row * dh) & (col < (row + 1) * dh)
    scale = dh ** -0.5

    cp_x.start()
    for u in range(_LW):
        _start(wq_el(u))
    cp_wr.start()
    cp_x.wait()
    x = x_buf[...].reshape(1, d).astype(jnp.float32)
    xn = jnp.broadcast_to(_layernorm(x), (_M, d)).astype(bf)
    acc_ref[...] = jnp.zeros_like(acc_ref)
    obd_ref[...] = jnp.zeros_like(obd_ref)

    def wq_loop(u, carry):
        _wait(wq_el(u))
        _start(wq_el(u + _LW))
        return carry

    def wq_wo_loop(u, carry):
        _wait(wq_el(u))
        _start(wo_el(u + _LW - nuq))
        return carry

    jax.lax.fori_loop(0, nuq - _LW, wq_loop, 0)
    jax.lax.fori_loop(nuq - _LW, nuq, wq_wo_loop, 0)

    epq = (nuo - _LW) // npair

    def wo_loop(j, carry):
        for i in range(epq):
            u = j * epq + i
            _wait(wo_el(u))
            _start(wo_el(u + _LW))
        q = jnp.dot(xn, wq_buf[j].reshape(d, gd), preferred_element_type=jnp.float32)
        q_ref[j] = jnp.where(diag, q, 0.0).astype(bf)
        return carry

    jax.lax.fori_loop(0, npair, wo_loop, 0)
    for u in range(epq * npair, nuo - _LW):
        _wait(wo_el(u))
        _start(wo_el(u + _LW))
    n_first = _LOOK * epb
    k = 0
    for i, u in enumerate(range(nuo - _LW, nuo)):
        _wait(wo_el(u))
        while k < -(-(i + 1) * n_first // _LW):
            _start(kv_el(0, k // epb, k % epb))
            k += 1

    def out_proj(pair, c0, cn):
        wo = wo_buf.at[pair // ppg, pl.ds(_hint((pair % ppg) * gd, 16), gd), :]
        acc_ref[:, c0:c0 + cn] += jnp.dot(obd_ref[...], wo[:, c0:c0 + cn], preferred_element_type=jnp.float32)

    def pair_loop(pair, carry):
        s, m, l = [None] * nb, [None] * nb, [None] * nb

        def block_softmax(b):
            sb = s[b] * scale
            m[b] = jnp.max(sb, axis=-1, keepdims=True)
            e = jnp.exp(sb - m[b])
            l[b] = jnp.sum(e, axis=-1, keepdims=True)
            p_ref[b] = e.astype(bf)

        o = None
        for pos in range(pb):
            for c in range(epb):
                _wait(kv_el(pair, pos, c))
                if pos + _LOOK < pb:
                    _start(kv_el(pair, pos + _LOOK, c))
                else:
                    @pl.when(pair < npair - 1)
                    def _():
                        _start(kv_el(pair + 1, pos + _LOOK - pb, c))

                    k = (pos + _LOOK - pb) * epb + c
                    if k < n_ffn_early:
                        @pl.when(pair == npair - 1)
                        def _():
                            _start(ffn_els[k])
            blk = kv_buf[pos % _NR]
            b = pos % nb
            if pos < d // 128:
                out_proj(jnp.maximum(pair - 1, 0), pos * 128, 128)
            if pos < nb:
                s[b] = jnp.dot(q_ref[pair], blk, preferred_element_type=jnp.float32)
                if b > 0:
                    block_softmax(b - 1)
            else:
                r = jax.lax.dot_general(p_ref[b], blk, (((1,), (1,)), ((), ())),
                                        preferred_element_type=jnp.float32)
                if b == 0:
                    block_softmax(nb - 1)
                    mx = functools.reduce(jnp.maximum, m)
                    fs = [jnp.exp(mb - mx) for mb in m]
                    linv = 1.0 / functools.reduce(jnp.add, [fb * lb for fb, lb in zip(fs, l)])
                r = r * fs[b]
                o = r if o is None else o + r
        obd_ref[...] = jnp.where(diag, o * linv, 0.0).astype(bf)
        return carry

    jax.lax.fori_loop(0, npair, pair_loop, 0)

    out_proj(npair - 1, 0, d)
    x = x_buf[...].reshape(1, d).astype(jnp.float32)
    h = x + jnp.sum(acc_ref[...], axis=0, keepdims=True)
    hn = _layernorm(h)
    hb = jnp.broadcast_to(hn, (_M, d)).astype(bf)
    cp_wr.wait()
    wr = wr_buf[...].reshape(1, d).astype(jnp.float32)
    gate = jax.nn.sigmoid(jnp.sum(hn * wr, axis=-1, keepdims=True))

    pending = ffn_els[n_ffn_early:]

    def consume(els):
        for el in els:
            _wait(el)
            if pending:
                _start(pending.pop(0))

    consume(wg_els)
    g = jnp.dot(hb, wg_buf[...], preferred_element_type=jnp.float32)
    g = g * jax.nn.sigmoid(g)
    consume(wu_els)
    u = jnp.dot(hb, wu_buf[...], preferred_element_type=jnp.float32)
    a = (g * u).astype(bf)
    y = jnp.zeros((_M, d), jnp.float32)
    eps = kslab // sum(_DOWN_SPLIT)
    for i in range(f // kslab):
        consume(wd_els[i * eps:(i + 1) * eps])
        y = y + jnp.dot(a[:, i * kslab:(i + 1) * kslab], wd_buf[i * kslab:(i + 1) * kslab, :],
                        preferred_element_type=jnp.float32)
    assert not pending
    out = h + hn + y[0:1, :] * gate
    o_ref[...] = out.reshape(o_ref.shape).astype(o_ref.dtype)


def _compiler_params():
    kw = dict(vmem_limit_bytes=64 * 1024 * 1024)
    if hasattr(pltpu.CompilerParams, "disable_semaphore_checks"):
        kw["disable_semaphore_checks"] = True
    return pltpu.CompilerParams(**kw)


@jax.jit
def pallas_sequential_preLN__sliding_block_cached__moe_arch_mod__decode_kernel(
    A_x: jax.Array,
    A_k_cache: jax.Array,
    A_v_cache: jax.Array,
    A_wq: jax.Array,
    A_wo: jax.Array,
    B_x: jax.Array,
    B_w_r: jax.Array,
    B_w_gate: jax.Array,
    B_w_up: jax.Array,
    B_w_down: jax.Array,
):
    b, sq, d = A_x.shape
    _, hkv, sk, dh = A_k_cache.shape
    assert b == 1 and sq == 1 and hkv == _HQ
    w = min(4096, max(256, sk // 4))
    f = B_w_gate.shape[1]
    gd = _G * dh
    npair = _HQ // _G
    bf = jnp.bfloat16

    kt = jnp.swapaxes(A_k_cache, 2, 3).reshape(hkv * dh, sk)
    vt = jnp.swapaxes(A_v_cache, 2, 3).reshape(hkv * dh, sk)
    wq3 = A_wq.reshape(_GQ, d // _GQ, hkv * dh)
    wo3 = A_wo.reshape(_GO, hkv * dh // _GO, d)

    any_spec = pl.BlockSpec(memory_space=pl.ANY)
    return pl.pallas_call(
        functools.partial(_kernel, dh=dh, sk=sk, w=w),
        in_specs=[any_spec] * 9,
        out_specs=pl.BlockSpec(memory_space=pltpu.VMEM),
        out_shape=jax.ShapeDtypeStruct(A_x.shape, A_x.dtype),
        scratch_shapes=[
            pltpu.VMEM(A_x.shape, bf),
            pltpu.VMEM(B_w_r.shape, bf),
            pltpu.VMEM((_NR, gd, _BC), bf),
            pltpu.VMEM((npair, _GQ, d // _GQ, gd), bf),
            pltpu.VMEM((_GO, hkv * dh // _GO, d), bf),
            pltpu.VMEM((d, f), bf),
            pltpu.VMEM((d, f), bf),
            pltpu.VMEM((f, d), bf),
            pltpu.VMEM((_M, d), jnp.float32),
            pltpu.VMEM((_M, gd), bf),
            pltpu.VMEM((w // _BC, _M, _BC), bf),
            pltpu.VMEM((npair, _M, gd), bf),
            pltpu.SemaphoreType.DMA((2,)),
            pltpu.SemaphoreType.DMA((_NR,)),
            pltpu.SemaphoreType.DMA((4,)),
            pltpu.SemaphoreType.DMA((f // 128,)),
        ],
        compiler_params=_compiler_params(),
    )(A_x, kt, vt, wq3, wo3, B_w_r, B_w_gate, B_w_up, B_w_down)
```
